```python
import os as _os
_os.environ.setdefault("JAX_PLATFORMS", "cpu")
import jax
import jax.numpy as jnp

def _softmax(x, axis=-1):
    return jax.nn.softmax(x, axis=axis)
def _gelu(x):
    return jax.nn.gelu(x, approximate=True)
def _silu(x):
    return jax.nn.silu(x)
def _sigmoid(x):
    return jax.nn.sigmoid(x)
def _layernorm(x, axis=-1, eps=1e-5):
    m = jnp.mean(x, axis=axis, keepdims=True)
    v = jnp.var(x, axis=axis, keepdims=True)
    return (x - m) / jnp.sqrt(v + eps)
def _scatter_add(tgt, idx, src, axis=0):
    return tgt.at[idx].add(src)
def _segment_sum(src, seg, n):
    return jax.ops.segment_sum(src, seg, n)
class _Rng:
    def __init__(self, key):
        self._k = key
    def _next(self):
        self._k, sub = jax.random.split(self._k)
        return sub
    def normal(self, shape):
        return jax.random.normal(self._next(), shape, dtype=jnp.bfloat16)
    def randint(self, lo, hi, shape):
        return jax.random.randint(self._next(), shape, lo, hi, dtype=jnp.int32)
    def uniform(self, shape, lo=0.0, hi=1.0):
        return jax.random.uniform(self._next(), shape, jnp.bfloat16, lo, hi)
    def permutation(self, n):
        return jax.random.permutation(self._next(), n)


kernel_name = 'parallel_sum__softmax_full_mha__moe_arch_mod__prompt'

def setup_inputs():
    _rng = _Rng(jax.random.key(int.from_bytes(__import__("os").urandom(4), "little")))
    _w = (lambda a: (lambda t: t.astype(jnp.bfloat16) if jnp.issubdtype(t.dtype, jnp.floating) else t)(jnp.asarray(a)))
    def _A_setup():
        B, S, D = 1, 2048, 512
        return {
            "x": _w((lambda *s: _rng.normal(s) * 0.05)(B, S, D)),
            "wqkv": _w((lambda *s: _rng.normal(s) * 0.1)(D, 3 * D)),
            "wo": _w((lambda *s: _rng.normal(s) * 0.05)(D, D)),
        }
    _A_in = _A_setup()

    def _B_setup():
        B, S, D, F, C = 1, 2048, 512, 1792, 1
        return {
            "x": _w((lambda *s: _rng.normal(s) * 0.05)(B, S, D)),
            "w_r": _w((lambda *s: _rng.normal(s) * 1.6)(D)),
            "w_gate": _w((lambda *s: _rng.normal(s) * 0.1)(D, F)),
            "w_up": _w((lambda *s: _rng.normal(s) * 0.1)(D, F)),
            "w_down": _w((lambda *s: _rng.normal(s) * 0.1)(F, D)),
        }
    _B_in = _B_setup()

    return {
        "A_x": _A_in["x"],
        "A_wqkv": _A_in["wqkv"],
        "A_wo": _A_in["wo"],
        "B_x": _B_in["x"],
        "B_w_r": _B_in["w_r"],
        "B_w_gate": _B_in["w_gate"],
        "B_w_up": _B_in["w_up"],
        "B_w_down": _B_in["w_down"],
    }

def reference(A_x, A_wqkv, A_wo, B_x, B_w_r, B_w_gate, B_w_up, B_w_down):
    def _A_ref(x, wqkv, wo):
        B, S, D = x.shape
        H = 32; Dh = D // H
        qkv = (lambda x, *d: x.transpose(*d))((x @ wqkv).reshape(B, S, 3, H, Dh), 2, 0, 3, 1, 4)
        q, k, v = qkv[0], qkv[1], qkv[2]
        scale = Dh ** -0.5
        scores = jnp.einsum("bhqd,bhkd->bhqk", q, k) * scale
        p = _softmax(scores, axis=-1)
        o = jnp.einsum("bhqk,bhkd->bhqd", p, v)
        return (lambda x, *d: x.transpose(*d))(o, 0, 2, 1, 3).reshape(B, S, D) @ wo

    def _B_ref(x, w_r, w_gate, w_up, w_down):
        B, S, D = x.shape
        C = 1
        r = x @ w_r
        idx = jnp.argsort(-r, axis=-1)[:, :C]
        idx_e = jnp.repeat(idx.reshape(B, C, 1), D, axis=2)
        x_sel = jnp.take_along_axis(x, idx_e, axis=1)
        g = _silu(x_sel @ w_gate)
        u = x_sel @ w_up
        y = (g * u) @ w_down
        r_sel = _sigmoid(jnp.take_along_axis(r, idx, axis=1))
        y = y * r_sel.reshape(B, C, 1)
        b_off = (jnp.arange(B) * S).reshape(B, 1)
        flat_idx = (idx + b_off).reshape(B * C)
        zero = (x * 0.0).reshape(B * S, D)
        upd = _scatter_add(zero, flat_idx, y.reshape(B * C, D), axis=0)
        return x + upd.reshape(B, S, D)

    x = A_x
    xn = _layernorm(x, axis=-1)
    return x + _A_ref(xn, A_wqkv, A_wo) + _B_ref(xn, B_w_r, B_w_gate, B_w_up, B_w_down)
```

```python
import jax
import jax.numpy as jnp
import numpy as np
from jax import lax
import jax.experimental.pallas as pl
import jax.experimental.pallas.tpu as pltpu

S = 2048
D = 512
H = 32
DH = 16
F = 1792
BQ = 512
KC = 128
NQ = S // BQ
NITEM = H * NQ
TC = 512
NTC = S // TC
QSCALE = float(DH ** -0.5 * np.log2(np.e))
BF = jnp.bfloat16
F32 = jnp.float32

_NT = (((1,), (1,)), ((), ()))
_TN = (((0,), (0,)), ((), ()))


def _kernel(x_hbm, wqkv_hbm, wo_hbm, wr_ref, wg_hbm, wu_hbm, wd_hbm, o_hbm,
            x_v, wqkv_v, wo_v, wg_v, wu_v, wd_v, xn_v, k_v, qt_v, vt_v, ot_v,
            p0, p1, r_v, out_v, sems):
    def x_cp(c):
        return pltpu.make_async_copy(x_hbm.at[pl.ds(c * TC, TC)], x_v.at[pl.ds(c * TC, TC)], sems.at[c])
    wqkv_cp = pltpu.make_async_copy(wqkv_hbm, wqkv_v, sems.at[NTC])
    wo_cp = pltpu.make_async_copy(wo_hbm, wo_v, sems.at[NTC + 1])
    wg_cp = pltpu.make_async_copy(wg_hbm, wg_v, sems.at[NTC + 2])
    wu_cp = pltpu.make_async_copy(wu_hbm, wu_v, sems.at[NTC + 3])
    wd_cp = pltpu.make_async_copy(wd_hbm, wd_v, sems.at[NTC + 4])
    x_cp(0).start()
    wqkv_cp.start()
    for c in range(1, NTC):
        x_cp(c).start()
    wo_cp.start()
    wg_cp.start()
    wu_cp.start()
    wd_cp.start()

    wr = wr_ref[...].astype(F32)
    wqT = None
    for c in range(NTC):
        x_cp(c).wait()
        x = x_v[pl.ds(c * TC, TC), :].astype(F32)
        m = jnp.mean(x, axis=-1, keepdims=True)
        xm = x - m
        var = jnp.mean(xm * xm, axis=-1, keepdims=True)
        xn = (xm * lax.rsqrt(var + 1e-5)).astype(BF)
        xn_v[pl.ds(c * TC, TC), :] = xn
        r_v[pl.ds(c * TC, TC), :] = jnp.sum(xn.astype(F32) * wr, axis=-1, keepdims=True)
        if c == 0:
            wqkv_cp.wait()
            wqT = wqkv_v[:, 0:D].T
            wvT = wqkv_v[:, 2 * D:3 * D].T
        k = jnp.dot(xn, wqkv_v[:, D:2 * D], preferred_element_type=F32).astype(BF)
        for g in range(4):
            k_v[g, pl.ds(c * TC, TC), :] = k[:, g * 128:(g + 1) * 128]
        qt = lax.dot_general(wqT, xn, _NT, preferred_element_type=F32) * QSCALE
        qt_v[:, pl.ds(c * TC, TC)] = qt.astype(BF)
        vt = lax.dot_general(wvT, xn, _NT, preferred_element_type=F32)
        vt_v[:, pl.ds(c * TC, TC)] = vt.astype(BF)

    def getq(i):
        qb = i // H
        h = i % H
        g = h // 8
        hh = h % 8
        qoff = pl.multiple_of(qb * BQ, BQ)
        goff = pl.multiple_of(g * 128, 128)
        qt_all = qt_v[pl.ds(goff, 128), pl.ds(qoff, BQ)]
        rows = lax.broadcasted_iota(jnp.int32, (128, BQ), 0)
        return jnp.where((rows // DH) == hh, qt_all, jnp.zeros_like(qt_all)), g

    def AB(iA, pA, iB, pB, lB, bad, doA=True, doB=True):
        if doA:
            qt, g = getq(iA)
        if doB:
            hoff = pl.multiple_of((iB % H) * DH, DH)
            qoffB = pl.multiple_of((iB // H) * BQ, BQ)
        l = jnp.zeros((8, BQ), F32)
        acc = jnp.zeros((DH, BQ), F32)
        for kc in range(S // KC):
            if doA:
                k = k_v[g, kc * KC:(kc + 1) * KC, :]
                s = jnp.dot(k, qt, preferred_element_type=F32)
                p = jnp.exp2(s)
                l = l + jnp.sum(p.reshape(KC // 8, 8, BQ), axis=0)
                pA[kc * KC:(kc + 1) * KC, :] = p.astype(BF)
            if doB:
                vt = vt_v[pl.ds(hoff, DH), kc * KC:(kc + 1) * KC]
                acc = acc + jnp.dot(vt, pB[kc * KC:(kc + 1) * KC, :], preferred_element_type=F32)
        if doB:
            lsum = jnp.sum(lB, axis=0, keepdims=True)
            ok_l = jnp.logical_and(lsum >= 2.0 ** -60, lsum <= 2.0 ** 100)
            ok_a = jnp.abs(acc) <= 2.0 ** 120
            badl = jnp.where(ok_l, 0.0, 1.0)
            bada = jnp.where(ok_a, 0.0, 1.0)
            bad = jnp.maximum(bad, jnp.maximum(badl, jnp.max(bada, axis=0, keepdims=True)))
            ot_v[pl.ds(hoff, DH), pl.ds(qoffB, BQ)] = (acc / lsum).astype(BF)
        return l, bad

    bad = jnp.zeros((1, BQ), F32)
    l, _ = AB(0, p0, 0, p1, None, bad, doB=False)

    def body(j, carry):
        l, bad = carry
        i = 2 * j
        l1, bad = AB(i + 1, p1, i, p0, l, bad)
        l2, bad = AB(i + 2, p0, i + 1, p1, l1, bad)
        return l2, bad

    l, bad = lax.fori_loop(0, NITEM // 2 - 1, body, (l, bad))
    l1, bad = AB(NITEM - 1, p1, NITEM - 2, p0, l, bad)
    _, bad = AB(0, p0, NITEM - 1, p1, l1, bad, doA=False)

    @pl.when(jnp.max(bad) > 0.0)
    def _():
        def item(i, _):
            qt, g = getq(i)
            hoff = pl.multiple_of((i % H) * DH, DH)
            qoff = pl.multiple_of((i // H) * BQ, BQ)

            def mx(kc, m):
                koff = pl.multiple_of(kc * KC, KC)
                s = jnp.dot(k_v[g, pl.ds(koff, KC), :], qt, preferred_element_type=F32)
                return jnp.maximum(m, jnp.max(s, axis=0, keepdims=True))
            m = lax.fori_loop(0, S // KC, mx, jnp.full((1, BQ), -jnp.inf, F32))

            def pv(kc, carry):
                l, acc = carry
                koff = pl.multiple_of(kc * KC, KC)
                s = jnp.dot(k_v[g, pl.ds(koff, KC), :], qt, preferred_element_type=F32)
                p = jnp.exp2(s - m)
                l = l + jnp.sum(p, axis=0, keepdims=True)
                vt = vt_v[pl.ds(hoff, DH), pl.ds(koff, KC)]
                acc = acc + jnp.dot(vt, p.astype(BF), preferred_element_type=F32)
                return l, acc
            l, acc = lax.fori_loop(0, S // KC, pv, (jnp.zeros((1, BQ), F32), jnp.zeros((DH, BQ), F32)))
            ot_v[pl.ds(hoff, DH), pl.ds(qoff, BQ)] = (acc / l).astype(BF)
            return 0
        lax.fori_loop(0, NITEM, item, 0)

    r = r_v[...].astype(BF).astype(F32)
    rmax = jnp.max(r, axis=0, keepdims=True)
    ids = lax.broadcasted_iota(jnp.int32, (S, 1), 0)
    idx = jnp.min(jnp.where(r == rmax, ids, S), axis=0, keepdims=True)
    onehot = (lax.broadcasted_iota(jnp.int32, (8, S), 1) == idx).astype(BF)
    xsel = jnp.dot(onehot, xn_v[...], preferred_element_type=F32).astype(BF)
    wg_cp.wait()
    wu_cp.wait()
    wd_cp.wait()
    gate = jnp.dot(xsel, wg_v[...], preferred_element_type=F32)
    up = jnp.dot(xsel, wu_v[...], preferred_element_type=F32)
    act = (gate * jax.nn.sigmoid(gate) * up).astype(BF)
    y = jnp.dot(act, wd_v[...], preferred_element_type=F32)
    y = y[0:1, :] * jax.nn.sigmoid(rmax)

    wo_cp.wait()
    def out_cp(c):
        return pltpu.make_async_copy(out_v.at[pl.ds(c * TC, TC)], o_hbm.at[pl.ds(c * TC, TC)], sems.at[c])
    for c in range(NTC):
        ot = ot_v[:, pl.ds(c * TC, TC)]
        a = lax.dot_general(ot, wo_v[...], _TN, preferred_element_type=F32)
        rows = c * TC + lax.broadcasted_iota(jnp.int32, (TC, 1), 0)
        upd = jnp.where(rows == idx, y, 0.0)
        res = x_v[pl.ds(c * TC, TC), :].astype(F32) + a + (xn_v[pl.ds(c * TC, TC), :].astype(F32) + upd)
        out_v[pl.ds(c * TC, TC), :] = res.astype(BF)
        out_cp(c).start()
    for c in range(NTC):
        out_cp(c).wait()


@jax.jit
def pallas_parallel_sum__softmax_full_mha__moe_arch_mod__prompt_kernel(
    A_x, A_wqkv, A_wo, B_x, B_w_r, B_w_gate, B_w_up, B_w_down,
):
    del B_x
    x = A_x.reshape(S, D)
    wr = B_w_r.reshape(1, D)
    any_spec = pl.BlockSpec(memory_space=pl.ANY)
    out = pl.pallas_call(
        _kernel,
        out_shape=jax.ShapeDtypeStruct((S, D), BF),
        in_specs=[any_spec, any_spec, any_spec, pl.BlockSpec(memory_space=pltpu.VMEM), any_spec, any_spec, any_spec],
        out_specs=any_spec,
        scratch_shapes=[
            pltpu.VMEM((S, D), BF),
            pltpu.VMEM((D, 3 * D), BF),
            pltpu.VMEM((D, D), BF),
            pltpu.VMEM((D, F), BF),
            pltpu.VMEM((D, F), BF),
            pltpu.VMEM((F, D), BF),
            pltpu.VMEM((S, D), BF),
            pltpu.VMEM((4, S, 128), BF),
            pltpu.VMEM((D, S), BF),
            pltpu.VMEM((D, S), BF),
            pltpu.VMEM((D, S), BF),
            pltpu.VMEM((S, BQ), BF),
            pltpu.VMEM((S, BQ), BF),
            pltpu.VMEM((S, 1), F32),
            pltpu.VMEM((S, D), BF),
            pltpu.SemaphoreType.DMA((NTC + 5,)),
        ],
        compiler_params=pltpu.CompilerParams(vmem_limit_bytes=100 * 1024 * 1024),
    )(x, A_wqkv, A_wo, wr, B_w_gate, B_w_up, B_w_down)
    return out.reshape(1, S, D)
```

```python
import jax
import jax.numpy as jnp
import numpy as np
from jax import lax
import jax.experimental.pallas as pl
import jax.experimental.pallas.tpu as pltpu

S = 2048
D = 512
H = 32
DH = 16
F = 1792
BQ = 512
KC = 128
NQ = S // BQ
NITEM = H * NQ
TC = 512
NTC = S // TC
UNROLL = 6
OUT_CHUNKS = (512, 512, 512, 256, 128, 128)
QSCALE = float(DH ** -0.5 * np.log2(np.e))
BF = jnp.bfloat16
F32 = jnp.float32

_NT = (((1,), (1,)), ((), ()))
_TN = (((0,), (0,)), ((), ()))


def _kernel(x_hbm, wqkv_hbm, wo_hbm, wr_ref, wg_hbm, wu_hbm, wd_hbm, o_hbm,
            x_v, wqkv_v, wo_v, wg_v, wu_v, wd_v, xn_v, k_v, qt_v, vt_v, ot_v,
            p0, p1, qm_v, out_v, sems):
    def x_cp(c):
        return pltpu.make_async_copy(x_hbm.at[pl.ds(c * TC, TC)], x_v.at[pl.ds(c * TC, TC)], sems.at[c])

    def w_cp(j):
        return pltpu.make_async_copy(wqkv_hbm.at[:, pl.ds(j * D, D)], wqkv_v.at[:, pl.ds(j * D, D)], sems.at[NTC + j])
    wo_cp = pltpu.make_async_copy(wo_hbm, wo_v, sems.at[NTC + 3])
    wg_cp = pltpu.make_async_copy(wg_hbm, wg_v, sems.at[NTC + 4])
    wu_cp = pltpu.make_async_copy(wu_hbm, wu_v, sems.at[NTC + 5])
    wd_cp = pltpu.make_async_copy(wd_hbm, wd_v, sems.at[NTC + 6])
    x_cp(0).start()
    w_cp(1).start()
    x_cp(1).start()
    w_cp(0).start()
    w_cp(2).start()
    x_cp(2).start()
    x_cp(3).start()

    def ln(c):
        x = x_v[pl.ds(c * TC, TC), :].astype(F32)
        m = jnp.mean(x, axis=-1, keepdims=True)
        xm = x - m
        var = jnp.mean(xm * xm, axis=-1, keepdims=True)
        xn = (xm * lax.rsqrt(var + 1e-5)).astype(BF)
        xn_v[pl.ds(c * TC, TC), :] = xn
        return xn

    def kproj(c, xn):
        k = jnp.dot(xn, wqkv_v[:, D:2 * D], preferred_element_type=F32).astype(BF)
        for g in range(4):
            k_v[g, pl.ds(c * TC, TC), :] = k[:, g * 128:(g + 1) * 128]

    def qvproj(c, xn, wqvT):
        qv = lax.dot_general(wqvT, xn, _NT, preferred_element_type=F32)
        qt_v[:, pl.ds(c * TC, TC)] = (qv[0:D] * QSCALE).astype(BF)
        vt_v[:, pl.ds(c * TC, TC)] = qv[D:2 * D].astype(BF)
        return qv[2 * D:2 * D + 8]

    x_cp(0).wait()
    xn0 = ln(0)
    w_cp(1).wait()
    kproj(0, xn0)
    x_cp(1).wait()
    xn1 = ln(1)
    kproj(1, xn1)
    w_cp(0).wait()
    w_cp(2).wait()
    wg_cp.start()
    wu_cp.start()
    wd_cp.start()
    wo_cp.start()
    wr16 = jnp.broadcast_to(wr_ref[...].reshape(1, D), (16, D))
    wqvT = jnp.concatenate([wqkv_v[:, 0:D].T, wqkv_v[:, 2 * D:3 * D].T, wr16], axis=0)
    rs = [qvproj(0, xn0, wqvT)]
    x_cp(2).wait()
    x_cp(3).wait()
    rs.append(qvproj(1, xn1, wqvT))
    for c in (2, 3):
        xn = ln(c)
        kproj(c, xn)
        rs.append(qvproj(c, xn, wqvT))
    r = jnp.concatenate(rs, axis=1).astype(BF).astype(F32)
    rmax = jnp.max(r, axis=1, keepdims=True)
    ids = lax.broadcasted_iota(jnp.int32, (8, S), 1)
    idx = jnp.min(jnp.where(r == rmax, ids, S), axis=1, keepdims=True)
    onehot = (ids == idx).astype(BF)

    def shr(a, n):
        return lax.shift_right_logical(a, jnp.int32(n)) if not isinstance(a, int) else a >> n

    def getq(i):
        qb = shr(i, 5)
        g = shr(i, 3) & 3
        hh = i & 7
        qoff = pl.multiple_of(qb * BQ, BQ)
        goff = pl.multiple_of(g * 128, 128)
        qt_all = qt_v[pl.ds(goff, 128), pl.ds(qoff, BQ)]
        rows = lax.broadcasted_iota(jnp.int32, (128, BQ), 0)
        return jnp.where(lax.shift_right_logical(rows, jnp.int32(4)) == hh, qt_all, jnp.zeros_like(qt_all)), g

    def AB(iA, pA, iB, pB, lB, bad, doA=True, doB=True, hooks=None, qt=None):
        if doA:
            if qt is None:
                qt, g = getq(iA)
            else:
                g = shr(iA, 3) & 3
        if doB:
            hoff = pl.multiple_of((iB & (H - 1)) * DH, DH)
            qoffB = pl.multiple_of(shr(iB, 5) * BQ, BQ)
        l = jnp.zeros((8, BQ), F32)
        acc = jnp.zeros((DH, BQ), F32)
        for kc in range(S // KC):
            if hooks is not None and kc in hooks:
                hooks[kc]()
            if doA:
                k = k_v[g, kc * KC:(kc + 1) * KC, :]
                s = jnp.dot(k, qt, preferred_element_type=F32)
                p = jnp.exp2(s)
                l = l + jnp.sum(p.reshape(KC // 8, 8, BQ), axis=0)
                pA[kc * KC:(kc + 1) * KC, :] = p.astype(BF)
            if doB:
                vt = vt_v[pl.ds(hoff, DH), kc * KC:(kc + 1) * KC]
                acc = acc + jnp.dot(vt, pB[kc * KC:(kc + 1) * KC, :], preferred_element_type=F32)
        if doB:
            lsum = jnp.sum(lB, axis=0, keepdims=True)
            ok_l = jnp.logical_and(lsum >= 2.0 ** -60, lsum <= 2.0 ** 100)
            ok_a = jnp.abs(acc) <= 2.0 ** 120
            badl = jnp.where(ok_l, 0.0, 1.0)
            bada = jnp.where(ok_a, 0.0, 1.0)
            bad = jnp.maximum(bad, jnp.maximum(badl, jnp.max(bada, axis=0, keepdims=True)))
            ot_v[pl.ds(hoff, DH), pl.ds(qoffB, BQ)] = (acc / lsum).astype(BF)
        return l, bad


    wg_cp.wait()
    wu_cp.wait()
    wd_cp.wait()
    wo_cp.wait()
    st = {}

    def fx(j):
        def f():
            part = jnp.dot(onehot[:, j * 512:(j + 1) * 512], xn_v[j * 512:(j + 1) * 512, :], preferred_element_type=F32)
            st["xs"] = part if j == 0 else st["xs"] + part
            if j == 3:
                st["xsel"] = st["xs"].astype(BF)
        return f

    def fg(name, w, lo, hi):
        def f():
            st.setdefault(name, []).append(jnp.dot(st["xsel"], w[:, lo:hi], preferred_element_type=F32))
        return f

    def fd(lo, hi, last):
        def f():
            if "act" not in st:
                gate = jnp.concatenate(st["gate"], axis=1)
                up = jnp.concatenate(st["up"], axis=1)
                st["act"] = (gate * jax.nn.sigmoid(gate) * up).astype(BF)
            part = jnp.dot(st["act"][:, lo:hi], wd_v[lo:hi, :], preferred_element_type=F32)
            st["ya"] = part if lo == 0 else st["ya"] + part
            if last:
                st["y"] = (st["ya"] * jax.nn.sigmoid(rmax))[0:1, :]
        return f

    hooks = {0: fx(0), 1: fx(1), 2: fx(2), 3: fx(3),
             5: fg("gate", wg_v, 0, 512), 6: fg("up", wu_v, 0, 512),
             7: fg("gate", wg_v, 512, 1024), 8: fg("up", wu_v, 512, 1024),
             9: fg("gate", wg_v, 1024, 1408), 10: fg("up", wu_v, 1024, 1408),
             11: fg("gate", wg_v, 1408, F), 12: fg("up", wu_v, 1408, F),
             14: fd(0, 896, False), 15: fd(896, F, True)}

    bufs = (p0, p1)
    bad = jnp.zeros((1, BQ), F32)
    l, _ = AB(0, p0, 0, p1, None, bad, doB=False, hooks=hooks)
    y = st["y"]

    qm_v[...] = getq(1)[0]

    def body(j, carry):
        l, bad = carry
        for u in range(UNROLL):
            i = UNROLL * j + u
            qt = qm_v[...] if u == 0 else None
            l, bad = AB(i + 1, bufs[(u + 1) % 2], i, bufs[u % 2], l, bad, qt=qt)
            if u == 1:
                qm_v[...] = getq(jnp.minimum(UNROLL * (j + 1) + 1, NITEM - 1))[0]
        return l, bad

    nloop = (NITEM - 1) // UNROLL
    l, bad = lax.fori_loop(0, nloop, body, (l, bad))
    for i in range(nloop * UNROLL, NITEM - 1):
        l, bad = AB(i + 1, bufs[(i + 1) % 2], i, bufs[i % 2], l, bad)
    _, bad = AB(0, p0, NITEM - 1, bufs[(NITEM - 1) % 2], l, bad, doA=False)

    @pl.when(jnp.max(bad) > 0.0)
    def _():
        def item(i, _):
            qt, g = getq(i)
            hoff = pl.multiple_of((i & (H - 1)) * DH, DH)
            qoff = pl.multiple_of(shr(i, 5) * BQ, BQ)

            def mx(kc, m):
                koff = pl.multiple_of(kc * KC, KC)
                s = jnp.dot(k_v[g, pl.ds(koff, KC), :], qt, preferred_element_type=F32)
                return jnp.maximum(m, jnp.max(s, axis=0, keepdims=True))
            m = lax.fori_loop(0, S // KC, mx, jnp.full((1, BQ), -jnp.inf, F32))

            def pv(kc, carry):
                l, acc = carry
                koff = pl.multiple_of(kc * KC, KC)
                s = jnp.dot(k_v[g, pl.ds(koff, KC), :], qt, preferred_element_type=F32)
                p = jnp.exp2(s - m)
                l = l + jnp.sum(p, axis=0, keepdims=True)
                vt = vt_v[pl.ds(hoff, DH), pl.ds(koff, KC)]
                acc = acc + jnp.dot(vt, p.astype(BF), preferred_element_type=F32)
                return l, acc
            l, acc = lax.fori_loop(0, S // KC, pv, (jnp.zeros((1, BQ), F32), jnp.zeros((DH, BQ), F32)))
            ot_v[pl.ds(hoff, DH), pl.ds(qoff, BQ)] = (acc / l).astype(BF)
            return 0
        lax.fori_loop(0, NITEM, item, 0)

    cps = []
    off = 0
    for c, n in enumerate(OUT_CHUNKS):
        ot = ot_v[:, pl.ds(off, n)]
        a = lax.dot_general(ot, wo_v[...], _TN, preferred_element_type=F32)
        rows = off + lax.broadcasted_iota(jnp.int32, (n, 1), 0)
        upd = jnp.where(rows == idx[0:1, :], y, 0.0)
        res = x_v[pl.ds(off, n), :].astype(F32) + a + (xn_v[pl.ds(off, n), :].astype(F32) + upd)
        out_v[pl.ds(off, n), :] = res.astype(BF)
        cp = pltpu.make_async_copy(out_v.at[pl.ds(off, n)], o_hbm.at[pl.ds(off, n)], sems.at[c])
        cp.start()
        cps.append(cp)
        off += n
    for cp in cps:
        cp.wait()


@jax.jit
def pallas_parallel_sum__softmax_full_mha__moe_arch_mod__prompt_kernel(
    A_x, A_wqkv, A_wo, B_x, B_w_r, B_w_gate, B_w_up, B_w_down,
):
    del B_x
    x = A_x.reshape(S, D)
    any_spec = pl.BlockSpec(memory_space=pl.ANY)
    out = pl.pallas_call(
        _kernel,
        out_shape=jax.ShapeDtypeStruct((S, D), BF),
        in_specs=[any_spec, any_spec, any_spec, pl.BlockSpec(memory_space=pltpu.VMEM), any_spec, any_spec, any_spec],
        out_specs=any_spec,
        scratch_shapes=[
            pltpu.VMEM((S, D), BF),
            pltpu.VMEM((D, 3 * D), BF),
            pltpu.VMEM((D, D), BF),
            pltpu.VMEM((D, F), BF),
            pltpu.VMEM((D, F), BF),
            pltpu.VMEM((F, D), BF),
            pltpu.VMEM((S, D), BF),
            pltpu.VMEM((4, S, 128), BF),
            pltpu.VMEM((D, S), BF),
            pltpu.VMEM((D, S), BF),
            pltpu.VMEM((D, S), BF),
            pltpu.VMEM((S, BQ), BF),
            pltpu.VMEM((S, BQ), BF),
            pltpu.VMEM((128, BQ), BF),
            pltpu.VMEM((S, D), BF),
            pltpu.SemaphoreType.DMA((NTC + 7,)),
        ],
        compiler_params=pltpu.CompilerParams(vmem_limit_bytes=100 * 1024 * 1024),
    )(x, A_wqkv, A_wo, B_w_r, B_w_gate, B_w_up, B_w_down)
    return out.reshape(1, S, D)
```

```python
import jax
import jax.numpy as jnp
import numpy as np
from jax import lax
import jax.experimental.pallas as pl
import jax.experimental.pallas.tpu as pltpu

S = 2048
D = 512
H = 32
DH = 16
F = 1792
BQ = 512
KC = 128
NQ = S // BQ
NITEM = H * NQ
TC = 512
NTC = S // TC
UNROLL = 6
OUT_CHUNKS = (512, 512, 512, 256, 128, 128)
QSCALE = float(DH ** -0.5 * np.log2(np.e))
BF = jnp.bfloat16
F32 = jnp.float32

_NT = (((1,), (1,)), ((), ()))
_TN = (((0,), (0,)), ((), ()))


def _kernel(x_hbm, wqkv_hbm, wo_hbm, wr_ref, wg_hbm, wu_hbm, wd_hbm, o_hbm,
            x_v, wqkv_v, wo_v, wg_v, wu_v, wd_v, xn_v, k_v, qt_v, vt_v, ot_v,
            p0, p1, qm_v, out_v, sems):
    def x_cp(c):
        return pltpu.make_async_copy(x_hbm.at[pl.ds(c * TC, TC)], x_v.at[pl.ds(c * TC, TC)], sems.at[c])

    def w_cp(j):
        return pltpu.make_async_copy(wqkv_hbm.at[:, pl.ds(j * D, D)], wqkv_v.at[:, pl.ds(j * D, D)], sems.at[NTC + j])
    wo_cp = pltpu.make_async_copy(wo_hbm, wo_v, sems.at[NTC + 3])
    wg_cp = pltpu.make_async_copy(wg_hbm, wg_v, sems.at[NTC + 4])
    wu_cp = pltpu.make_async_copy(wu_hbm, wu_v, sems.at[NTC + 5])
    wd_cp = pltpu.make_async_copy(wd_hbm, wd_v, sems.at[NTC + 6])
    x_cp(0).start()
    w_cp(1).start()
    x_cp(1).start()
    w_cp(0).start()
    w_cp(2).start()
    x_cp(2).start()
    x_cp(3).start()

    def ln(c):
        x = x_v[pl.ds(c * TC, TC), :].astype(F32)
        m = jnp.mean(x, axis=-1, keepdims=True)
        xm = x - m
        var = jnp.mean(xm * xm, axis=-1, keepdims=True)
        xn = (xm * lax.rsqrt(var + 1e-5)).astype(BF)
        xn_v[pl.ds(c * TC, TC), :] = xn
        return xn

    def kproj(c, xn):
        k = jnp.dot(xn, wqkv_v[:, D:2 * D], preferred_element_type=F32).astype(BF)
        for g in range(4):
            k_v[g, pl.ds(c * TC, TC), :] = k[:, g * 128:(g + 1) * 128]

    def qvproj(c, xn, wqvT):
        qv = lax.dot_general(wqvT, xn, _NT, preferred_element_type=F32)
        qt_v[:, pl.ds(c * TC, TC)] = (qv[0:D] * QSCALE).astype(BF)
        vt_v[:, pl.ds(c * TC, TC)] = qv[D:2 * D].astype(BF)
        return qv[2 * D:2 * D + 8]

    x_cp(0).wait()
    xn0 = ln(0)
    w_cp(1).wait()
    kproj(0, xn0)
    x_cp(1).wait()
    xn1 = ln(1)
    kproj(1, xn1)
    w_cp(0).wait()
    w_cp(2).wait()
    wg_cp.start()
    wu_cp.start()
    wd_cp.start()
    wo_cp.start()
    wr16 = jnp.broadcast_to(wr_ref[...].reshape(1, D), (16, D))
    wqvT = jnp.concatenate([wqkv_v[:, 0:D].T, wqkv_v[:, 2 * D:3 * D].T, wr16], axis=0)
    rs = [qvproj(0, xn0, wqvT)]
    x_cp(2).wait()
    x_cp(3).wait()
    rs.append(qvproj(1, xn1, wqvT))
    for c in (2, 3):
        xn = ln(c)
        kproj(c, xn)
        rs.append(qvproj(c, xn, wqvT))
    r = jnp.concatenate(rs, axis=1).astype(BF).astype(F32)
    rmax = jnp.max(r, axis=1, keepdims=True)
    ids = lax.broadcasted_iota(jnp.int32, (8, S), 1)
    idx = jnp.min(jnp.where(r == rmax, ids, S), axis=1, keepdims=True)
    onehot = (ids == idx).astype(BF)

    vmax = jnp.max(jnp.abs(vt_v[...].astype(F32)), axis=1, keepdims=True)
    ok_v = jnp.logical_or(vmax == 0.0, vmax >= 2.0 ** -30)
    vbad = jnp.max(jnp.where(ok_v, 0.0, 1.0), axis=0, keepdims=True)

    def shr(a, n):
        return lax.shift_right_logical(a, jnp.int32(n)) if not isinstance(a, int) else a >> n

    def getq(i):
        qb = shr(i, 5)
        g = shr(i, 3) & 3
        hh = i & 7
        qoff = pl.multiple_of(qb * BQ, BQ)
        goff = pl.multiple_of(g * 128, 128)
        qt_all = qt_v[pl.ds(goff, 128), pl.ds(qoff, BQ)]
        rows = lax.broadcasted_iota(jnp.int32, (128, BQ), 0)
        return jnp.where(lax.shift_right_logical(rows, jnp.int32(4)) == hh, qt_all, jnp.zeros_like(qt_all)), g

    def AB(iA, pA, iB, pB, lB, bad, doA=True, doB=True, hooks=None, qt=None):
        if doA:
            if qt is None:
                qt, g = getq(iA)
            else:
                g = shr(iA, 3) & 3
        if doB:
            hoff = pl.multiple_of((iB & (H - 1)) * DH, DH)
            qoffB = pl.multiple_of(shr(iB, 5) * BQ, BQ)
        l = jnp.zeros((8, BQ), F32)
        acc = jnp.zeros((DH, BQ), F32)
        for kc in range(S // KC):
            if hooks is not None and kc in hooks:
                hooks[kc]()
            if doA:
                k = k_v[g, kc * KC:(kc + 1) * KC, :]
                s = jnp.dot(k, qt, preferred_element_type=F32)
                p = jnp.exp2(s)
                l = l + jnp.sum(p.reshape(KC // 8, 8, BQ), axis=0)
                pA[kc * KC:(kc + 1) * KC, :] = p.astype(BF)
            if doB:
                vt = vt_v[pl.ds(hoff, DH), kc * KC:(kc + 1) * KC]
                acc = acc + jnp.dot(vt, pB[kc * KC:(kc + 1) * KC, :], preferred_element_type=F32)
        if doB:
            lsum = jnp.sum(lB, axis=0, keepdims=True)
            ok_l = jnp.logical_and(lsum >= 2.0 ** -60, lsum <= 2.0 ** 100)
            ok_a = jnp.abs(acc) <= 2.0 ** 120
            badl = jnp.where(ok_l, 0.0, 1.0)
            bada = jnp.where(ok_a, 0.0, 1.0)
            bad = jnp.maximum(bad, jnp.maximum(badl, jnp.max(bada, axis=0, keepdims=True)))
            ot_v[pl.ds(hoff, DH), pl.ds(qoffB, BQ)] = (acc / lsum).astype(BF)
        return l, bad


    wg_cp.wait()
    wu_cp.wait()
    wd_cp.wait()
    wo_cp.wait()
    st = {}

    def fx(j):
        def f():
            part = jnp.dot(onehot[:, j * 512:(j + 1) * 512], xn_v[j * 512:(j + 1) * 512, :], preferred_element_type=F32)
            st["xs"] = part if j == 0 else st["xs"] + part
            if j == 3:
                st["xsel"] = st["xs"].astype(BF)
        return f

    def fg(name, w, lo, hi):
        def f():
            st.setdefault(name, []).append(jnp.dot(st["xsel"], w[:, lo:hi], preferred_element_type=F32))
        return f

    def fd(lo, hi, last):
        def f():
            if "act" not in st:
                gate = jnp.concatenate(st["gate"], axis=1)
                up = jnp.concatenate(st["up"], axis=1)
                st["act"] = (gate * jax.nn.sigmoid(gate) * up).astype(BF)
            part = jnp.dot(st["act"][:, lo:hi], wd_v[lo:hi, :], preferred_element_type=F32)
            st["ya"] = part if lo == 0 else st["ya"] + part
            if last:
                st["y"] = (st["ya"] * jax.nn.sigmoid(rmax))[0:1, :]
        return f

    hooks = {0: fx(0), 1: fx(1), 2: fx(2), 3: fx(3),
             5: fg("gate", wg_v, 0, 512), 6: fg("up", wu_v, 0, 512),
             7: fg("gate", wg_v, 512, 1024), 8: fg("up", wu_v, 512, 1024),
             9: fg("gate", wg_v, 1024, 1408), 10: fg("up", wu_v, 1024, 1408),
             11: fg("gate", wg_v, 1408, F), 12: fg("up", wu_v, 1408, F),
             14: fd(0, 896, False), 15: fd(896, F, True)}

    bufs = (p0, p1)
    bad = jnp.zeros((1, BQ), F32)
    l, _ = AB(0, p0, 0, p1, None, bad, doB=False, hooks=hooks)
    y = st["y"]

    qm_v[...] = getq(1)[0]

    def body(j, carry):
        l, bad = carry
        for u in range(UNROLL):
            i = UNROLL * j + u
            qt = qm_v[...] if u == 0 else None
            l, bad = AB(i + 1, bufs[(u + 1) % 2], i, bufs[u % 2], l, bad, qt=qt)
            if u == 1:
                qm_v[...] = getq(jnp.minimum(UNROLL * (j + 1) + 1, NITEM - 1))[0]
        return l, bad

    nloop = (NITEM - 1) // UNROLL
    l, bad = lax.fori_loop(0, nloop, body, (l, bad))
    for i in range(nloop * UNROLL, NITEM - 1):
        l, bad = AB(i + 1, bufs[(i + 1) % 2], i, bufs[i % 2], l, bad)
    _, bad = AB(0, p0, NITEM - 1, bufs[(NITEM - 1) % 2], l, bad, doA=False)

    bad = jnp.maximum(bad, vbad)

    @pl.when(jnp.max(bad) > 0.0)
    def _():
        def item(i, _):
            qt, g = getq(i)
            hoff = pl.multiple_of((i & (H - 1)) * DH, DH)
            qoff = pl.multiple_of(shr(i, 5) * BQ, BQ)

            def mx(kc, m):
                koff = pl.multiple_of(kc * KC, KC)
                s = jnp.dot(k_v[g, pl.ds(koff, KC), :], qt, preferred_element_type=F32)
                return jnp.maximum(m, jnp.max(s, axis=0, keepdims=True))
            m = lax.fori_loop(0, S // KC, mx, jnp.full((1, BQ), -jnp.inf, F32))

            def pv(kc, carry):
                l, acc = carry
                koff = pl.multiple_of(kc * KC, KC)
                s = jnp.dot(k_v[g, pl.ds(koff, KC), :], qt, preferred_element_type=F32)
                p = jnp.exp2(s - m)
                l = l + jnp.sum(p, axis=0, keepdims=True)
                vt = vt_v[pl.ds(hoff, DH), pl.ds(koff, KC)]
                acc = acc + jnp.dot(vt, p.astype(BF), preferred_element_type=F32)
                return l, acc
            l, acc = lax.fori_loop(0, S // KC, pv, (jnp.zeros((1, BQ), F32), jnp.zeros((DH, BQ), F32)))
            ot_v[pl.ds(hoff, DH), pl.ds(qoff, BQ)] = (acc / l).astype(BF)
            return 0
        lax.fori_loop(0, NITEM, item, 0)

    cps = []
    off = 0
    for c, n in enumerate(OUT_CHUNKS):
        ot = ot_v[:, pl.ds(off, n)]
        a = lax.dot_general(ot, wo_v[...], _TN, preferred_element_type=F32)
        rows = off + lax.broadcasted_iota(jnp.int32, (n, 1), 0)
        upd = jnp.where(rows == idx[0:1, :], y, 0.0)
        res = x_v[pl.ds(off, n), :].astype(F32) + a + (xn_v[pl.ds(off, n), :].astype(F32) + upd)
        out_v[pl.ds(off, n), :] = res.astype(BF)
        cp = pltpu.make_async_copy(out_v.at[pl.ds(off, n)], o_hbm.at[pl.ds(off, n)], sems.at[c])
        cp.start()
        cps.append(cp)
        off += n
    for cp in cps:
        cp.wait()


@jax.jit
def pallas_parallel_sum__softmax_full_mha__moe_arch_mod__prompt_kernel(
    A_x, A_wqkv, A_wo, B_x, B_w_r, B_w_gate, B_w_up, B_w_down,
):
    del B_x
    x = A_x.reshape(S, D)
    any_spec = pl.BlockSpec(memory_space=pl.ANY)
    out = pl.pallas_call(
        _kernel,
        out_shape=jax.ShapeDtypeStruct((S, D), BF),
        in_specs=[any_spec, any_spec, any_spec, pl.BlockSpec(memory_space=pltpu.VMEM), any_spec, any_spec, any_spec],
        out_specs=any_spec,
        scratch_shapes=[
            pltpu.VMEM((S, D), BF),
            pltpu.VMEM((D, 3 * D), BF),
            pltpu.VMEM((D, D), BF),
            pltpu.VMEM((D, F), BF),
            pltpu.VMEM((D, F), BF),
            pltpu.VMEM((F, D), BF),
            pltpu.VMEM((S, D), BF),
            pltpu.VMEM((4, S, 128), BF),
            pltpu.VMEM((D, S), BF),
            pltpu.VMEM((D, S), BF),
            pltpu.VMEM((D, S), BF),
            pltpu.VMEM((S, BQ), BF),
            pltpu.VMEM((S, BQ), BF),
            pltpu.VMEM((128, BQ), BF),
            pltpu.VMEM((S, D), BF),
            pltpu.SemaphoreType.DMA((NTC + 7,)),
        ],
        compiler_params=pltpu.CompilerParams(vmem_limit_bytes=100 * 1024 * 1024),
    )(x, A_wqkv, A_wo, B_w_r, B_w_gate, B_w_up, B_w_down)
    return out.reshape(1, S, D)
```
